```python
import os as _os
_os.environ.setdefault("JAX_PLATFORMS", "cpu")
import jax
import jax.numpy as jnp

def _softmax(x, axis=-1):
    return jax.nn.softmax(x, axis=axis)
def _gelu(x):
    return jax.nn.gelu(x, approximate=True)
def _silu(x):
    return jax.nn.silu(x)
def _sigmoid(x):
    return jax.nn.sigmoid(x)
def _layernorm(x, axis=-1, eps=1e-5):
    m = jnp.mean(x, axis=axis, keepdims=True)
    v = jnp.var(x, axis=axis, keepdims=True)
    return (x - m) / jnp.sqrt(v + eps)
def _scatter_add(tgt, idx, src, axis=0):
    return tgt.at[idx].add(src)
def _segment_sum(src, seg, n):
    return jax.ops.segment_sum(src, seg, n)
class _Rng:
    def __init__(self, key):
        self._k = key
    def _next(self):
        self._k, sub = jax.random.split(self._k)
        return sub
    def normal(self, shape):
        return jax.random.normal(self._next(), shape, dtype=jnp.bfloat16)
    def randint(self, lo, hi, shape):
        return jax.random.randint(self._next(), shape, lo, hi, dtype=jnp.int32)
    def uniform(self, shape, lo=0.0, hi=1.0):
        return jax.random.uniform(self._next(), shape, jnp.bfloat16, lo, hi)
    def permutation(self, n):
        return jax.random.permutation(self._next(), n)


kernel_name = 'standalone__dense_activation_silu__prompt'

def setup_inputs():
    _rng = _Rng(jax.random.key(int.from_bytes(__import__("os").urandom(4), "little")))
    _w = (lambda a: (lambda t: t.astype(jnp.bfloat16) if jnp.issubdtype(t.dtype, jnp.floating) else t)(jnp.asarray(a)))
    B, S, D, F = 1, 2048, 448, 1792
    return {
        "x": _w((lambda *s: _rng.normal(s) * 0.05)(B, S, D)),
        "w1": _w((lambda *s: _rng.normal(s) * 0.05)(D, F) * (D ** -0.5)),
        "w2": _w((lambda *s: _rng.normal(s) * 0.05)(F, D) * (F ** -0.5)),
    }

def reference(x, w1, w2):
    h = jnp.einsum("bsd,df->bsf", x, w1)
    h = _silu(h)
    out = jnp.einsum("bsf,fd->bsd", h, w2)
    return out
```

```python
import functools

import jax
import jax.numpy as jnp
import jax.experimental.pallas as pl
import jax.experimental.pallas.tpu as pltpu


def _ffn_kernel(x_ref, w1_ref, w2_ref, o_ref):
    h = jnp.dot(x_ref[...], w1_ref[...], preferred_element_type=jnp.float32)
    h = h * jax.nn.sigmoid(h)
    o = jnp.dot(h.astype(jnp.bfloat16), w2_ref[...],
                preferred_element_type=jnp.float32)
    o_ref[...] = o.astype(o_ref.dtype)


@jax.jit
def pallas_standalone__dense_activation_silu__prompt_kernel(
    x: jax.Array,
    w1: jax.Array,
    w2: jax.Array,
):
    B, S, D = x.shape
    F = w1.shape[1]
    M = B * S
    x2 = x.reshape(M, D)
    tm = 256
    out = pl.pallas_call(
        _ffn_kernel,
        grid=(M // tm,),
        in_specs=[
            pl.BlockSpec((tm, D), lambda i: (i, 0)),
            pl.BlockSpec((D, F), lambda i: (0, 0)),
            pl.BlockSpec((F, D), lambda i: (0, 0)),
        ],
        out_specs=pl.BlockSpec((tm, D), lambda i: (i, 0)),
        out_shape=jax.ShapeDtypeStruct((M, D), x.dtype),
        compiler_params=pltpu.CompilerParams(
            dimension_semantics=("arbitrary",),
            vmem_limit_bytes=64 * 1024 * 1024,
        ),
    )(x2, w1, w2)
    return out.reshape(B, S, D)
```

```python
import jax
import jax.numpy as jnp
import jax.experimental.pallas as pl
import jax.experimental.pallas.tpu as pltpu

D, S, F = 448, 2048, 1792
XO, W1O, W2O = 0, S, S + F
BF = jnp.bfloat16
F32 = jnp.float32
FB = 1024


def _startup_program():
    f3, t1, b3, b4 = 1280, 256, 64, 128
    return [
        ('W', [('w1', 384, 448, 0, t1)]),
        ('T', 384, 448, 0, t1),
        ('W', [('x', 384, 448, 0, 512), ('w1', 384, 448, t1, FB)]),
        ('T', 384, 448, t1, FB),
        ('P', 384, 448, 0, FB, 0, 512, 'set'),
        ('W', [('x', 384, 448, 512, 1024), ('w1', 0, 128, 0, FB),
               ('x', 0, 128, 0, 1024)]),
        ('P', 384, 448, 0, FB, 512, 1024, 'set'),
        ('T', 0, 128, 0, FB),
        ('P', 0, 128, 0, FB - b3, 0, 1024, 'add'),
        ('W', [('w1', 128, 384, 0, FB), ('x', 128, 384, 0, 1024),
               ('w1', 0, D, FB, f3)]),
        ('P', 0, 128, FB - b3, FB, 0, 1024, 'add'),
        ('T', 128, 384, 0, FB),
        ('P', 128, 384, 0, FB, 0, 1024, 'fin'),
        ('T', 0, D, FB, f3),
        ('M', FB, f3 - b4, 0, 1024),
        ('M', f3 - b4, f3, 0, 768),
        ('W', [('w1', 0, D, f3, F), ('w2', 0, D, 0, F), ('x', 0, D, 1024, S)]),
        ('M', f3 - b4, f3, 768, 1024),
        ('T', 0, D, f3, F),
        ('M', f3, F, 0, 1024),
    ]


_PROG = _startup_program()
_PIECES = [p for st in _PROG if st[0] == 'W' for p in st[1]]
_TILES = [(0, 512), (512, 512), (1024, 512), (1536, 256), (1792, 256)]
_OUT = [(0, D, c0, n) for (c0, n) in _TILES[:-1]] + [
    (0, 384, 1792, 256), (384, 64, 1792, 256)]


def _dot(a, b):
    return jnp.dot(a, b, preferred_element_type=F32)


def _silu(h):
    t = 0.5 * h
    return t + t * jnp.tanh(t)


def _ffn_kernel(xt_hbm, w1_hbm, w2t_hbm, o_hbm,
                in_v, w1t_v, part_v, act_v, o_v, in_sem, o_sem):
    srcs = {'x': (xt_hbm, XO), 'w1': (w1_hbm, W1O), 'w2': (w2t_hbm, W2O)}

    def in_copy(i):
        w, r0, r1, c0, c1 = _PIECES[i]
        src, off = srcs[w]
        return pltpu.make_async_copy(
            src.at[pl.ds(r0, r1 - r0), pl.ds(c0, c1 - c0)],
            in_v.at[pl.ds(r0, r1 - r0), pl.ds(off + c0, c1 - c0)],
            in_sem.at[i])

    def out_copy(i):
        r0, nr, c0, n = _OUT[i]
        return pltpu.make_async_copy(
            o_v.at[pl.ds(r0, nr), pl.ds(c0, n)],
            o_hbm.at[pl.ds(r0, nr), pl.ds(c0, n)],
            o_sem.at[i])

    def mm2(i, a):
        r0, nr, c0, n = _OUT[i]
        o = _dot(in_v[r0:r0 + nr, W2O:W2O + F], a)
        o_v[r0:r0 + nr, c0:c0 + n] = o.astype(BF)
        out_copy(i).start()

    for i in range(len(_PIECES)):
        in_copy(i).start()

    k = 0
    for st in _PROG:
        if st[0] == 'W':
            for _ in st[1]:
                in_copy(k).wait()
                k += 1
        elif st[0] == 'T':
            _, r0, r1, f0, f1 = st
            w1t_v[f0:f1, r0:r1] = in_v[r0:r1, W1O + f0:W1O + f1].T
        elif st[0] == 'P':
            _, r0, r1, f0, f1, s0, s1, mode = st
            h = _dot(w1t_v[f0:f1, r0:r1], in_v[r0:r1, XO + s0:XO + s1])
            if mode == 'set':
                part_v[f0:f1, s0:s1] = h
            elif mode == 'add':
                part_v[f0:f1, s0:s1] = part_v[f0:f1, s0:s1] + h
            else:
                act_v[f0:f1, s0:s1] = _silu(part_v[f0:f1, s0:s1] + h).astype(BF)
        else:
            _, f0, f1, s0, s1 = st
            h = _dot(w1t_v[f0:f1, :], in_v[:, XO + s0:XO + s1])
            act_v[f0:f1, s0:s1] = _silu(h).astype(BF)

    mm2(0, act_v[:, 0:512])
    mm2(1, act_v[:, 512:1024])
    for i in range(2, len(_TILES)):
        c0, n = _TILES[i]
        a = _silu(_dot(w1t_v[...], in_v[:, XO + c0:XO + c0 + n])).astype(BF)
        for j in range(i, i + 1 if i < len(_TILES) - 1 else len(_OUT)):
            mm2(j, a)

    for i in range(len(_OUT)):
        out_copy(i).wait()


@jax.jit
def pallas_standalone__dense_activation_silu__prompt_kernel(
    x: jax.Array,
    w1: jax.Array,
    w2: jax.Array,
):
    assert x.shape == (1, S, D) and w1.shape == (D, F) and w2.shape == (F, D)
    xt = x.reshape(S, D).T
    w2t = w2.T
    out_t = pl.pallas_call(
        _ffn_kernel,
        in_specs=[pl.BlockSpec(memory_space=pl.ANY)] * 3,
        out_specs=pl.BlockSpec(memory_space=pl.ANY),
        out_shape=jax.ShapeDtypeStruct((D, S), x.dtype),
        scratch_shapes=[
            pltpu.VMEM((D, S + 2 * F), BF),
            pltpu.VMEM((F, D), BF),
            pltpu.VMEM((FB, 1024), F32),
            pltpu.VMEM((F, 1024), BF),
            pltpu.VMEM((D, S), BF),
            pltpu.SemaphoreType.DMA((len(_PIECES),)),
            pltpu.SemaphoreType.DMA((len(_OUT),)),
        ],
        compiler_params=pltpu.CompilerParams(
            vmem_limit_bytes=100 * 1024 * 1024,
            disable_semaphore_checks=True,
            disable_bounds_checks=True,
        ),
    )(xt, w1, w2t)
    return out_t.T.reshape(1, S, D)
```

```python
import jax
import jax.numpy as jnp
import jax.experimental.pallas as pl
import jax.experimental.pallas.tpu as pltpu

D, S, F = 448, 2048, 1792
HD, HF, HS = D // 2, F // 2, S // 2
XO, W1O, W2O = 0, S, S + F
BF = jnp.bfloat16
F32 = jnp.float32

CH = 512
NCH = HS // CH
T1 = 256
FILL_A, FILL_B = 256, 256
LAST = (144, 48, 32)

_GROUPS = [
    [('w1', 384, 448, HF, HF + T1)],
    [('x', 384, 448, 0, 512), ('x', 128, 192, 0, 512),
     ('w1', 384, 448, HF + T1, F)],
    [('x', 384, 448, 512, S), ('x', 128, 192, 512, HS),
     ('w1', 384, 448, 0, HF), ('w1', 128, 192, 0, HF)],
    [('w1', 192, 384, 0, F), ('x', 192, 384, 0, CH), ('x', 0, 128, 0, CH),
     ('w1', 0, 128, 0, F), ('x', 0, 384, HS, HS + CH),
     ('w1', 128, 192, HF, F)],
    [('w2', 0, D, 0, F), ('x', 192, 384, CH, HS), ('x', 0, 128, CH, HS),
     ('x', 0, 384, HS + CH, S)],
]
_PIECES = [p for g in _GROUPS for p in g]


def _out_blocks():
    outs = []
    for c in range(NCH):
        c0 = c * CH
        outs += [(HD, HD, c0, CH), (HD, HD, HS + c0, CH), (0, HD, HS + c0, CH)]
        rows = (HD,) if c < NCH - 1 else LAST
        r = 0
        for n in rows:
            outs.append((r, n, c0, CH))
            r += n
    return outs


_OUTS = _out_blocks()


def _dot(a, b):
    return jnp.dot(a, b, preferred_element_type=F32)


def _add(a, b):
    return (a.astype(F32) + b.astype(F32)).astype(BF)


def _sub(a, b):
    return (a.astype(F32) - b.astype(F32)).astype(BF)


def _padop(op, a, b):
    return jnp.concatenate([op(a[0:192], b), a[192:256]], axis=0)


def _silu(h):
    t = 0.5 * h
    return t + t * jnp.tanh(t)


def _ffn_kernel(xt_hbm, w1_hbm, w2t_hbm, o_hbm,
                in_v, p_v, b_v, o_v, in_sem, o_sem, pin_sem):
    srcs = {'x': (xt_hbm, XO), 'w1': (w1_hbm, W1O), 'w2': (w2t_hbm, W2O)}
    state = {'in': 0, 'out': 0}

    def in_copy(i):
        w, r0, r1, c0, c1 = _PIECES[i]
        src, off = srcs[w]
        return pltpu.make_async_copy(
            src.at[pl.ds(r0, r1 - r0), pl.ds(c0, c1 - c0)],
            in_v.at[pl.ds(r0, r1 - r0), pl.ds(off + c0, c1 - c0)],
            in_sem.at[i])

    def wait_group(g):
        for _ in _GROUPS[g]:
            in_copy(state['in']).wait()
            state['in'] += 1

    def out_copy(i):
        r0, nr, c0, n = _OUTS[i]
        return pltpu.make_async_copy(
            o_v.at[pl.ds(r0, nr), pl.ds(c0, n)],
            o_hbm.at[pl.ds(r0, nr), pl.ds(c0, n)],
            o_sem.at[i])

    def emit(v):
        i = state['out']
        state['out'] += 1
        r0, nr, c0, n = _OUTS[i]
        o_v[r0:r0 + nr, c0:c0 + n] = v.astype(BF)
        out_copy(i).start()

    def X(r0, r1, c0, c1):
        return in_v[r0:r1, XO + c0:XO + c1]

    def W1(r0, r1, c0, c1):
        return in_v[r0:r1, W1O + c0:W1O + c1]

    def W2(r0, r1, c0, c1):
        return in_v[r0:r1, W2O + c0:W2O + c1]

    def put_b(i, c0, v):
        for j in range(CH // 128):
            b_v[i, c0 // 128 + j] = v[:, j * 128:(j + 1) * 128].astype(BF)

    def get_b(i, c0):
        return jnp.concatenate(
            [b_v[i, c0 // 128 + j] for j in range(CH // 128)], axis=1)

    for i in range(len(_PIECES)):
        in_copy(i).start()

    p_v[3, 0:8, 0:128] = jnp.zeros((8, 128), F32)
    b_v[0, 0, 0:16, :] = jnp.zeros((16, 128), BF)
    pins = [
        pltpu.make_async_copy(p_v.at[3, pl.ds(0, 8), pl.ds(0, 128)],
                              p_v.at[3, pl.ds(8, 8), pl.ds(0, 128)],
                              pin_sem.at[0]),
        pltpu.make_async_copy(b_v.at[0, 0, pl.ds(0, 16), :],
                              b_v.at[0, 0, pl.ds(16, 16), :],
                              pin_sem.at[1]),
    ]
    for cp in pins:
        cp.start()

    P4, P5, P7 = 0, 1, 2

    wait_group(0)
    a4t = W1(384, 448, HF, HF + T1).T
    wait_group(1)
    a4t = jnp.concatenate([a4t, W1(384, 448, HF + T1, F).T], axis=0)
    p_v[P4, :, 0:512] = _dot(
        a4t, _sub(X(384, 448, 0, 512), X(128, 192, 0, 512)))
    wait_group(2)
    p_v[P4, :, 512:HS] = _dot(
        a4t, _sub(X(384, 448, 512, HS), X(128, 192, 512, HS)))
    a7t = _sub(W1(384, 448, 0, HF), W1(384, 448, HF, F)).T
    p_v[P7] = _dot(a7t, _add(X(384, 448, 0, HS), X(384, 448, HS, S)))
    a5t = _add(W1(128, 192, 0, HF), W1(384, 448, 0, HF)).T

    def m5_tail(r0, r1, c0, c1):
        p_v[P5, r0:r1, c0:c1] = _dot(a5t[r0:r1], X(384, 448, HS + c0, HS + c1))

    m5_tail(0, HF, 0, 512)
    m5_tail(0, HF - FILL_A - FILL_B, 512, HS)
    wait_group(3)
    m5_tail(HF - FILL_A - FILL_B, HF - FILL_B, 512, HS)

    def t_pair(u, v):
        t = jnp.concatenate([u, v], axis=1).T
        return t[0:HF], t[HF:F]

    def t_256(w):
        return jnp.concatenate(t_pair(w[0:128], w[128:256]), axis=1)

    A = {}
    A[4], A[7] = t_pair(W1(256, 384, HF, F),
                        _sub(W1(256, 384, 0, HF), W1(256, 384, HF, F)))
    A[5] = _add(W1(0, 128, 0, HF + 128), W1(256, 384, 0, HF + 128)).T[0:HF]
    A[1] = t_256(_padop(_add, W1(0, 256, 0, HF), W1(256, D, HF, F)))
    A[2] = t_256(_padop(_add, W1(0, 256, HF, F), W1(256, D, HF, F)))
    A[3] = t_256(W1(0, 256, 0, HF))
    A[6] = t_256(_sub(W1(0, 256, HF, F), W1(0, 256, 0, HF)))
    N = {}

    def chunk(c, first, second):
        a0, a1 = c * CH, (c + 1) * CH
        b0, b1 = HS + a0, HS + a1
        cs = slice(a0, a1)
        if first:
            p_v[P4, :, cs] = p_v[P4, :, cs] + _dot(
                A[4], _sub(X(256, 384, a0, a1), X(0, 128, a0, a1)))
            p_v[P7, :, cs] = p_v[P7, :, cs] + p_v[P4, :, cs] + _dot(
                A[7], _add(X(256, 384, a0, a1), X(256, 384, b0, b1)))
            p_v[P5, :, cs] = p_v[P5, :, cs] + _dot(
                A[5], X(256, 384, b0, b1))
            m1 = _dot(A[1], _padop(_add, X(0, 256, a0, a1), X(256, D, b0, b1)))
            g11 = _silu(p_v[P7, :, cs] - p_v[P5, :, cs] + m1)
            put_b(2, a0, g11)
            m2 = _dot(A[2], X(0, 256, a0, a1))
            g21 = _silu(m2 + p_v[P4, :, cs])
            put_b(4, a0, g21 - g11)
        if first and second:
            n2 = _dot(N[2], get_b(2, a0))
        if first:
            m3 = _dot(A[3], _padop(_sub, X(0, 256, b0, b1), X(256, D, b0, b1)))
            g12 = _silu(m3 + p_v[P5, :, cs])
            put_b(6, a0, g11 + g12)
        if second:
            n4 = _dot(N[4], get_b(4, a0))
            if not first:
                n2 = _dot(N[2], get_b(2, a0))
            emit(n2 + n4)
        if first:
            m6 = _dot(A[6], _add(X(0, 256, a0, a1), X(0, 256, b0, b1)))
            g22 = _silu(m1 - m2 + m3 + m6)
            put_b(1, a0, g11 + g22)
            put_b(3, a0, g12 - g22)
            put_b(5, a0, g22)
            put_b(7, a0, g21 + g22)
        if second:
            n6 = _dot(N[6], get_b(6, a0))
            n1 = _dot(N[1], get_b(1, a0))
            n3 = _dot(N[3], get_b(3, a0))
            emit(n1 - n2 + n3 + n6)
            n5 = _dot(N[5], get_b(5, a0))
            emit(n3 + n5)
            q = n1 + n4 - n5
            r = 0
            for n in ((HD,) if c < NCH - 1 else LAST):
                emit(q[r:r + n] + _dot(N[7][r:r + n], get_b(7, a0)))
                r += n

    chunk(0, True, False)
    m5_tail(HF - FILL_B, HF, 512, HS)
    wait_group(4)

    N[4] = W2(HD, D, HF, F)
    N[2] = _add(W2(HD, D, 0, HF), W2(HD, D, HF, F))
    N[6] = _sub(W2(HD, D, 0, HF), W2(0, HD, 0, HF))
    N[1] = _add(W2(0, HD, 0, HF), W2(HD, D, HF, F))
    N[3] = W2(0, HD, 0, HF)
    N[5] = _add(W2(0, HD, 0, HF), W2(0, HD, HF, F))
    N[7] = _sub(W2(0, HD, HF, F), W2(HD, D, HF, F))
    chunk(0, False, True)
    for c in range(1, NCH):
        chunk(c, True, True)

    for cp in pins:
        cp.wait()
    for i in range(len(_OUTS)):
        out_copy(i).wait()


@jax.jit
def pallas_standalone__dense_activation_silu__prompt_kernel(
    x: jax.Array,
    w1: jax.Array,
    w2: jax.Array,
):
    assert x.shape == (1, S, D) and w1.shape == (D, F) and w2.shape == (F, D)
    xt = x.reshape(S, D).T
    w2t = w2.T
    out_t = pl.pallas_call(
        _ffn_kernel,
        in_specs=[pl.BlockSpec(memory_space=pl.ANY)] * 3,
        out_specs=pl.BlockSpec(memory_space=pl.ANY),
        out_shape=jax.ShapeDtypeStruct((D, S), x.dtype),
        scratch_shapes=[
            pltpu.VMEM((D, S + 2 * F), BF),
            pltpu.VMEM((4, HF, HS), F32),
            pltpu.VMEM((8, HS // 128, HF, 128), BF),
            pltpu.VMEM((D, S), BF),
            pltpu.SemaphoreType.DMA((len(_PIECES),)),
            pltpu.SemaphoreType.DMA((len(_OUTS),)),
            pltpu.SemaphoreType.DMA((2,)),
        ],
        compiler_params=pltpu.CompilerParams(
            vmem_limit_bytes=110 * 1024 * 1024,
            disable_semaphore_checks=True,
            disable_bounds_checks=True,
        ),
    )(xt, w1, w2t)
    return out_t.T.reshape(1, S, D)
```

```python
import jax
import jax.numpy as jnp
import jax.experimental.pallas as pl
import jax.experimental.pallas.tpu as pltpu

D, S, F = 448, 2048, 1792
HD, HF, HS = D // 2, F // 2, S // 2
XO, W1O, W2O = 0, S, S + F
BF = jnp.bfloat16
F32 = jnp.float32

CH = 512
NCH = HS // CH
T1 = 256
FILL_A, FILL_B = 256, 128
LAST = (144, 48, 32)

_GROUPS = [
    [('w1', 384, 448, HF, HF + T1)],
    [('x', 384, 448, 0, 512), ('x', 128, 192, 0, 512),
     ('w1', 384, 448, HF + T1, F)],
    [('x', 384, 448, 512, S), ('x', 128, 192, 512, HS),
     ('w1', 384, 448, 0, HF), ('w1', 128, 192, 0, HF)],
    [('w1', 192, 384, 0, F), ('x', 192, 384, 0, CH), ('x', 0, 128, 0, CH),
     ('w1', 0, 128, 0, F), ('x', 256, 384, HS, HS + CH),
     ('w1', 128, 192, HF, F)],
    [('w2', 0, D, 0, F), ('x', 0, 256, HS, S), ('x', 192, 384, CH, HS),
     ('x', 0, 128, CH, HS), ('x', 256, 384, HS + CH, S)],
]
_PIECES = [p for g in _GROUPS for p in g]


def _out_blocks():
    outs = []
    for c in range(NCH):
        c0 = c * CH
        outs += [(HD, HD, c0, CH), (HD, HD, HS + c0, CH), (0, HD, HS + c0, CH)]
        r = 0
        for n in ((HD,) if c < NCH - 1 else LAST):
            outs.append((r, n, c0, CH))
            r += n
    return outs


_OUTS = _out_blocks()


def _dot(a, b):
    return jnp.dot(a, b, preferred_element_type=F32)


def _add(a, b):
    return (a.astype(F32) + b.astype(F32)).astype(BF)


def _sub(a, b):
    return (a.astype(F32) - b.astype(F32)).astype(BF)


def _padop(op, a, b):
    return jnp.concatenate([op(a[0:192], b), a[192:256]], axis=0)


def _silu(h):
    t = 0.5 * h
    return t + t * jnp.tanh(t)


def _ffn_kernel(xt_hbm, w1_hbm, w2t_hbm, o_hbm,
                in_v, p_v, b_v, o_v, in_sem, o_sem, pin_sem):
    srcs = {'x': (xt_hbm, XO), 'w1': (w1_hbm, W1O), 'w2': (w2t_hbm, W2O)}
    state = {'in': 0, 'out': 0}

    def in_copy(i):
        w, r0, r1, c0, c1 = _PIECES[i]
        src, off = srcs[w]
        return pltpu.make_async_copy(
            src.at[pl.ds(r0, r1 - r0), pl.ds(c0, c1 - c0)],
            in_v.at[pl.ds(r0, r1 - r0), pl.ds(off + c0, c1 - c0)],
            in_sem.at[i])

    def wait_group(g):
        for _ in _GROUPS[g]:
            in_copy(state['in']).wait()
            state['in'] += 1

    def out_copy(i):
        r0, nr, c0, n = _OUTS[i]
        return pltpu.make_async_copy(
            o_v.at[pl.ds(r0, nr), pl.ds(c0, n)],
            o_hbm.at[pl.ds(r0, nr), pl.ds(c0, n)],
            o_sem.at[i])

    def emit(v):
        i = state['out']
        state['out'] += 1
        r0, nr, c0, n = _OUTS[i]
        o_v[r0:r0 + nr, c0:c0 + n] = v.astype(BF)
        out_copy(i).start()

    def X(r0, r1, c0, c1):
        return in_v[r0:r1, XO + c0:XO + c1]

    def W1(r0, r1, c0, c1):
        return in_v[r0:r1, W1O + c0:W1O + c1]

    def W2(r0, r1, c0, c1):
        return in_v[r0:r1, W2O + c0:W2O + c1]

    def put_b(i, c0, v):
        for j in range(CH // 128):
            b_v[i, c0 // 128 + j] = v[:, j * 128:(j + 1) * 128].astype(BF)

    def get_b(i, c0):
        return jnp.concatenate(
            [b_v[i, c0 // 128 + j] for j in range(CH // 128)], axis=1)

    for i in range(len(_PIECES)):
        in_copy(i).start()

    p_v[3, 0:8, 0:128] = jnp.zeros((8, 128), F32)
    b_v[0, 0, 0:16, :] = jnp.zeros((16, 128), BF)
    pins = [
        pltpu.make_async_copy(p_v.at[3, pl.ds(0, 8), pl.ds(0, 128)],
                              p_v.at[3, pl.ds(8, 8), pl.ds(0, 128)],
                              pin_sem.at[0]),
        pltpu.make_async_copy(b_v.at[0, 0, pl.ds(0, 16), :],
                              b_v.at[0, 0, pl.ds(16, 16), :],
                              pin_sem.at[1]),
    ]
    for cp in pins:
        cp.start()

    P4, P5, P7 = 0, 1, 2

    wait_group(0)
    a4t = W1(384, 448, HF, HF + T1).T
    wait_group(1)
    a4t = jnp.concatenate([a4t, W1(384, 448, HF + T1, F).T], axis=0)
    p_v[P4, :, 0:512] = _dot(
        a4t, _sub(X(384, 448, 0, 512), X(128, 192, 0, 512)))
    wait_group(2)
    p_v[P4, :, 512:HS] = _dot(
        a4t, _sub(X(384, 448, 512, HS), X(128, 192, 512, HS)))
    a7t = _sub(W1(384, 448, 0, HF), W1(384, 448, HF, F)).T
    p_v[P7] = _dot(a7t, _add(X(384, 448, 0, HS), X(384, 448, HS, S)))
    a5t = _add(W1(128, 192, 0, HF), W1(384, 448, 0, HF)).T

    def m5_tail(r0, r1, c0, c1):
        p_v[P5, r0:r1, c0:c1] = _dot(a5t[r0:r1], X(384, 448, HS + c0, HS + c1))

    m5_tail(0, HF, 0, 512)
    m5_tail(0, HF - FILL_A - FILL_B, 512, HS)
    wait_group(3)
    m5_tail(HF - FILL_A - FILL_B, HF - FILL_B, 512, HS)

    def t_pair(u, v):
        t = jnp.concatenate([u, v], axis=1).T
        return t[0:HF], t[HF:F]

    def t_256(w):
        return jnp.concatenate(t_pair(w[0:128], w[128:256]), axis=1)

    A, N = {}, {}
    A[4], A[7] = t_pair(W1(256, 384, HF, F),
                        _sub(W1(256, 384, 0, HF), W1(256, 384, HF, F)))
    A[5] = _add(W1(0, 128, 0, HF + 128), W1(256, 384, 0, HF + 128)).T[0:HF]
    A[1] = t_256(_padop(_add, W1(0, 256, 0, HF), W1(256, D, HF, F)))
    A[2] = t_256(_padop(_add, W1(0, 256, HF, F), W1(256, D, HF, F)))

    def late_operands():
        m5_tail(HF - FILL_B, HF, 512, HS)
        wait_group(4)
        N[2] = _add(W2(HD, D, 0, HF), W2(HD, D, HF, F))
        N[4] = W2(HD, D, HF, F)
        N[6] = _sub(W2(HD, D, 0, HF), W2(0, HD, 0, HF))
        N[1] = _add(W2(0, HD, 0, HF), W2(HD, D, HF, F))
        N[3] = W2(0, HD, 0, HF)
        N[5] = _add(W2(0, HD, 0, HF), W2(0, HD, HF, F))
        N[7] = _sub(W2(0, HD, HF, F), W2(HD, D, HF, F))
        A[3] = t_256(W1(0, 256, 0, HF))
        A[6] = t_256(_sub(W1(0, 256, HF, F), W1(0, 256, 0, HF)))

    for c in range(NCH):
        a0, a1 = c * CH, (c + 1) * CH
        b0, b1 = HS + a0, HS + a1
        cs = slice(a0, a1)
        p_v[P4, :, cs] = p_v[P4, :, cs] + _dot(
            A[4], _sub(X(256, 384, a0, a1), X(0, 128, a0, a1)))
        p_v[P7, :, cs] = p_v[P7, :, cs] + p_v[P4, :, cs] + _dot(
            A[7], _add(X(256, 384, a0, a1), X(256, 384, b0, b1)))
        p_v[P5, :, cs] = p_v[P5, :, cs] + _dot(
            A[5], X(256, 384, b0, b1))
        m1 = _dot(A[1], _padop(_add, X(0, 256, a0, a1), X(256, D, b0, b1)))
        g11 = _silu(p_v[P7, :, cs] - p_v[P5, :, cs] + m1)
        put_b(2, a0, g11)
        m2 = _dot(A[2], X(0, 256, a0, a1))
        g21 = _silu(m2 + p_v[P4, :, cs])
        put_b(4, a0, g21 - g11)
        if c == 0:
            late_operands()
        n2 = _dot(N[2], get_b(2, a0))
        m3 = _dot(A[3], _padop(_sub, X(0, 256, b0, b1), X(256, D, b0, b1)))
        g12 = _silu(m3 + p_v[P5, :, cs])
        put_b(6, a0, g11 + g12)
        n4 = _dot(N[4], get_b(4, a0))
        emit(n2 + n4)
        m6 = _dot(A[6], _add(X(0, 256, a0, a1), X(0, 256, b0, b1)))
        g22 = _silu(m1 - m2 + m3 + m6)
        put_b(1, a0, g11 + g22)
        put_b(3, a0, g12 - g22)
        put_b(5, a0, g22)
        put_b(7, a0, g21 + g22)
        n6 = _dot(N[6], get_b(6, a0))
        n1 = _dot(N[1], get_b(1, a0))
        n3 = _dot(N[3], get_b(3, a0))
        emit(n1 - n2 + n3 + n6)
        n5 = _dot(N[5], get_b(5, a0))
        emit(n3 + n5)
        q = n1 + n4 - n5
        r = 0
        for n in ((HD,) if c < NCH - 1 else LAST):
            emit(q[r:r + n] + _dot(N[7][r:r + n], get_b(7, a0)))
            r += n

    for cp in pins:
        cp.wait()
    for i in range(len(_OUTS)):
        out_copy(i).wait()


@jax.jit
def pallas_standalone__dense_activation_silu__prompt_kernel(
    x: jax.Array,
    w1: jax.Array,
    w2: jax.Array,
):
    assert x.shape == (1, S, D) and w1.shape == (D, F) and w2.shape == (F, D)
    xt = x.reshape(S, D).T
    w2t = w2.T
    out_t = pl.pallas_call(
        _ffn_kernel,
        in_specs=[pl.BlockSpec(memory_space=pl.ANY)] * 3,
        out_specs=pl.BlockSpec(memory_space=pl.ANY),
        out_shape=jax.ShapeDtypeStruct((D, S), x.dtype),
        scratch_shapes=[
            pltpu.VMEM((D, S + 2 * F), BF),
            pltpu.VMEM((4, HF, HS), F32),
            pltpu.VMEM((8, HS // 128, HF, 128), BF),
            pltpu.VMEM((D, S), BF),
            pltpu.SemaphoreType.DMA((len(_PIECES),)),
            pltpu.SemaphoreType.DMA((len(_OUTS),)),
            pltpu.SemaphoreType.DMA((2,)),
        ],
        compiler_params=pltpu.CompilerParams(
            vmem_limit_bytes=110 * 1024 * 1024,
            disable_semaphore_checks=True,
            disable_bounds_checks=True,
        ),
    )(xt, w1, w2t)
    return out_t.T.reshape(1, S, D)
```

```python
import jax
import jax.numpy as jnp
import jax.experimental.pallas as pl
import jax.experimental.pallas.tpu as pltpu

D, S, F = 448, 2048, 1792
HD, HF, HS = D // 2, F // 2, S // 2
XO, W1O, W2O = 0, S, S + F
WIN = S + 2 * F
BF = jnp.bfloat16
F32 = jnp.float32

CH = 512
NCH = HS // CH
T1 = 256
FILL_A, FILL_B = 256, 128
LAST = (144, 48, 32)
SLAB, TIE = 64, 5
NMAX = 4 * NCH - 1

_GROUPS = [
    [('w1', 384, 448, HF, HF + T1)],
    [('x', 384, 448, 0, 512), ('x', 128, 192, 0, 512),
     ('w1', 384, 448, HF + T1, F)],
    [('x', 384, 448, 512, S), ('x', 128, 192, 512, HS),
     ('w1', 384, 448, 0, HF), ('w1', 128, 192, 0, HF)],
    [('w1', 192, 384, 0, F), ('x', 192, 384, 0, CH), ('x', 0, 128, 0, CH),
     ('w1', 0, 128, 0, F), ('x', 256, 384, HS, HS + CH),
     ('w1', 128, 192, HF, F)],
    [('w2', 0, D, 0, F), ('x', 0, 256, HS, S), ('x', 192, 384, CH, HS),
     ('x', 0, 128, CH, HS), ('x', 256, 384, HS + CH, S)],
]
_PIECES = [p for g in _GROUPS for p in g]


def _out_blocks():
    outs = []
    for c in range(NCH):
        c0 = c * CH
        outs += [(HD, HD, c0, CH), (HD, HD, HS + c0, CH), (0, HD, HS + c0, CH)]
        r = 0
        for n in ((HD,) if c < NCH - 1 else LAST):
            outs.append((r, n, c0, CH))
            r += n
    return outs


_OUTS = _out_blocks()


def _dot(a, b):
    return jnp.dot(a, b, preferred_element_type=F32)


def _add(a, b):
    return (a.astype(F32) + b.astype(F32)).astype(BF)


def _sub(a, b):
    return (a.astype(F32) - b.astype(F32)).astype(BF)


def _padop(op, a, b):
    return jnp.concatenate([op(a[0:192], b), a[192:256]], axis=0)


def _silu(h):
    t = 0.5 * h
    return t + t * jnp.tanh(t)


def _absmax8(v):
    return jnp.max(jnp.abs(v).reshape(v.shape[0] // 8, 8, v.shape[1]), axis=0)


def _ffn_kernel(xt_hbm, w1_hbm, w2t_hbm, o_hbm,
                in_v, p_v, b_v, o_v, st_v, w1t_v, acc_v,
                in_sem, o_sem, aux_sem):
    srcs = {'x': (xt_hbm, XO), 'w1': (w1_hbm, W1O), 'w2': (w2t_hbm, W2O)}
    state = {'in': 0, 'out': 0}

    def in_copy(i):
        w, r0, r1, c0, c1 = _PIECES[i]
        src, off = srcs[w]
        return pltpu.make_async_copy(
            src.at[pl.ds(r0, r1 - r0), pl.ds(c0, c1 - c0)],
            in_v.at[pl.ds(r0, r1 - r0), pl.ds(off + c0, c1 - c0)],
            in_sem.at[i])

    def wait_group(g):
        for _ in _GROUPS[g]:
            in_copy(state['in']).wait()
            state['in'] += 1

    def out_copy(i):
        r0, nr, c0, n = _OUTS[i]
        return pltpu.make_async_copy(
            o_v.at[pl.ds(r0, nr), pl.ds(c0, n)],
            o_hbm.at[pl.ds(r0, nr), pl.ds(c0, n)],
            o_sem.at[i])

    def emit(v):
        i = state['out']
        state['out'] += 1
        r0, nr, c0, n = _OUTS[i]
        o_v[r0:r0 + nr, c0:c0 + n] = v.astype(BF)
        out_copy(i).start()
        if i < NMAX:
            st_v[8:16, i * CH:(i + 1) * CH] = _absmax8(v)

    def X(r0, r1, c0, c1):
        return in_v[r0:r1, XO + c0:XO + c1]

    def W1(r0, r1, c0, c1):
        return in_v[r0:r1, W1O + c0:W1O + c1]

    def W2(r0, r1, c0, c1):
        return in_v[r0:r1, W2O + c0:W2O + c1]

    def put_b(i, c0, v):
        for j in range(CH // 128):
            b_v[i, c0 // 128 + j] = v[:, j * 128:(j + 1) * 128].astype(BF)

    def get_b(i, c0):
        return jnp.concatenate(
            [b_v[i, c0 // 128 + j] for j in range(CH // 128)], axis=1)

    stat_jobs = [(r, c) for c in range(0, WIN, 256) for r in range(0, D, SLAB)]

    def stats(v):
        for c in range(CH // 128):
            for r in range(0, HD // 8, TIE):
                if not stat_jobs:
                    return
                r0, c0 = stat_jobs.pop(0)
                z = jnp.minimum(
                    jnp.abs(v[8 * r:8 * r + 8, 128 * c:128 * c + 128]), 0.0)
                u = in_v[r0:r0 + SLAB, c0:c0 + 256].astype(F32)
                u = jnp.sum((u * u).reshape(SLAB // 8, 8, 256), axis=0)
                u = u + jnp.concatenate([z, z], axis=1)
                if r0:
                    u = u + st_v[0:8, c0:c0 + 256]
                st_v[0:8, c0:c0 + 256] = u

    for i in range(len(_PIECES)):
        in_copy(i).start()

    p_v[3, 0:8, 0:128] = jnp.zeros((8, 128), F32)
    b_v[0, 0, 0:16, :] = jnp.zeros((16, 128), BF)
    st_v[24:32, 0:128] = jnp.zeros((8, 128), F32)
    pins = [
        pltpu.make_async_copy(p_v.at[3, pl.ds(0, 8), pl.ds(0, 128)],
                              p_v.at[3, pl.ds(8, 8), pl.ds(0, 128)],
                              aux_sem.at[0]),
        pltpu.make_async_copy(b_v.at[0, 0, pl.ds(0, 16), :],
                              b_v.at[0, 0, pl.ds(16, 16), :],
                              aux_sem.at[1]),
        pltpu.make_async_copy(st_v.at[pl.ds(24, 8), pl.ds(0, 128)],
                              st_v.at[pl.ds(24, 8), pl.ds(128, 128)],
                              aux_sem.at[2]),
    ]
    for cp in pins:
        cp.start()

    P4, P5, P7 = 0, 1, 2

    wait_group(0)
    a4t = W1(384, 448, HF, HF + T1).T
    wait_group(1)
    a4t = jnp.concatenate([a4t, W1(384, 448, HF + T1, F).T], axis=0)
    p_v[P4, :, 0:512] = _dot(
        a4t, _sub(X(384, 448, 0, 512), X(128, 192, 0, 512)))
    wait_group(2)
    p_v[P4, :, 512:HS] = _dot(
        a4t, _sub(X(384, 448, 512, HS), X(128, 192, 512, HS)))
    a7t = _sub(W1(384, 448, 0, HF), W1(384, 448, HF, F)).T
    p_v[P7] = _dot(a7t, _add(X(384, 448, 0, HS), X(384, 448, HS, S)))
    a5t = _add(W1(128, 192, 0, HF), W1(384, 448, 0, HF)).T

    def m5_tail(r0, r1, c0, c1):
        p_v[P5, r0:r1, c0:c1] = _dot(a5t[r0:r1], X(384, 448, HS + c0, HS + c1))

    m5_tail(0, HF, 0, 512)
    m5_tail(0, HF - FILL_A - FILL_B, 512, HS)
    wait_group(3)
    m5_tail(HF - FILL_A - FILL_B, HF - FILL_B, 512, HS)

    def t_pair(u, v):
        t = jnp.concatenate([u, v], axis=1).T
        return t[0:HF], t[HF:F]

    def t_256(w):
        return jnp.concatenate(t_pair(w[0:128], w[128:256]), axis=1)

    A, N = {}, {}
    A[4], A[7] = t_pair(W1(256, 384, HF, F),
                        _sub(W1(256, 384, 0, HF), W1(256, 384, HF, F)))
    A[5] = _add(W1(0, 128, 0, HF + 128), W1(256, 384, 0, HF + 128)).T[0:HF]
    A[1] = t_256(_padop(_add, W1(0, 256, 0, HF), W1(256, D, HF, F)))
    A[2] = t_256(_padop(_add, W1(0, 256, HF, F), W1(256, D, HF, F)))

    def late_operands():
        m5_tail(HF - FILL_B, HF, 512, HS)
        wait_group(4)
        N[2] = _add(W2(HD, D, 0, HF), W2(HD, D, HF, F))
        N[4] = W2(HD, D, HF, F)
        N[6] = _sub(W2(HD, D, 0, HF), W2(0, HD, 0, HF))
        N[1] = _add(W2(0, HD, 0, HF), W2(HD, D, HF, F))
        N[3] = W2(0, HD, 0, HF)
        N[5] = _add(W2(0, HD, 0, HF), W2(0, HD, HF, F))
        N[7] = _sub(W2(0, HD, HF, F), W2(HD, D, HF, F))
        A[3] = t_256(W1(0, 256, 0, HF))
        A[6] = t_256(_sub(W1(0, 256, HF, F), W1(0, 256, 0, HF)))

    for c in range(NCH):
        a0, a1 = c * CH, (c + 1) * CH
        b0, b1 = HS + a0, HS + a1
        cs = slice(a0, a1)
        p_v[P4, :, cs] = p_v[P4, :, cs] + _dot(
            A[4], _sub(X(256, 384, a0, a1), X(0, 128, a0, a1)))
        p_v[P7, :, cs] = p_v[P7, :, cs] + p_v[P4, :, cs] + _dot(
            A[7], _add(X(256, 384, a0, a1), X(256, 384, b0, b1)))
        p_v[P5, :, cs] = p_v[P5, :, cs] + _dot(
            A[5], X(256, 384, b0, b1))
        m1 = _dot(A[1], _padop(_add, X(0, 256, a0, a1), X(256, D, b0, b1)))
        g11 = _silu(p_v[P7, :, cs] - p_v[P5, :, cs] + m1)
        put_b(2, a0, g11)
        m2 = _dot(A[2], X(0, 256, a0, a1))
        g21 = _silu(m2 + p_v[P4, :, cs])
        put_b(4, a0, g21 - g11)
        if c == 0:
            late_operands()
        n2 = _dot(N[2], get_b(2, a0))
        m3 = _dot(A[3], _padop(_sub, X(0, 256, b0, b1), X(256, D, b0, b1)))
        g12 = _silu(m3 + p_v[P5, :, cs])
        put_b(6, a0, g11 + g12)
        n4 = _dot(N[4], get_b(4, a0))
        emit(n2 + n4)
        m6 = _dot(A[6], _add(X(0, 256, a0, a1), X(0, 256, b0, b1)))
        g22 = _silu(m1 - m2 + m3 + m6)
        put_b(1, a0, g11 + g22)
        put_b(3, a0, g12 - g22)
        put_b(5, a0, g22)
        put_b(7, a0, g21 + g22)
        n6 = _dot(N[6], get_b(6, a0))
        stats(n6)
        n1 = _dot(N[1], get_b(1, a0))
        st_v[16:24, cs] = _absmax8(n1)
        stats(n1)
        n3 = _dot(N[3], get_b(3, a0))
        stats(n3)
        emit(n1 - n2 + n3 + n6)
        n5 = _dot(N[5], get_b(5, a0))
        stats(n5)
        emit(n3 + n5)
        q = n1 + n4 - n5
        r = 0
        for n in ((HD,) if c < NCH - 1 else LAST):
            emit(q[r:r + n] + _dot(N[7][r:r + n], get_b(7, a0)))
            r += n
    assert not stat_jobs

    for cp in pins:
        cp.wait()
    for i in range(NMAX):
        out_copy(i).wait()

    def amax(v):
        return jnp.max(jnp.max(v, axis=0, keepdims=True), axis=1, keepdims=True)

    sq = jnp.sum(st_v[0:8, :], axis=0, keepdims=True)
    nx = jnp.max(sq[:, XO:XO + S], axis=1, keepdims=True)
    nw1 = jnp.max(sq[:, W1O:W1O + F], axis=1, keepdims=True)
    nw2 = jnp.sum(sq[:, W2O:W2O + F], axis=1, keepdims=True)
    omax = amax(st_v[8:16, 0:NMAX * CH])
    scale = jnp.maximum(
        jnp.sqrt(nx) * jnp.sqrt(nw1) * jnp.sqrt(nw2) * (0.8 / D),
        0.25 * amax(st_v[16:24, 0:HS]))
    safe = jnp.max(jnp.where(scale <= omax, 1, 0).astype(jnp.int32))

    for i in range(NMAX, len(_OUTS)):
        out_copy(i).wait()

    @pl.when(safe == 0)
    def _classical():
        def transpose_w1(j, carry):
            f0 = pl.multiple_of(j * 256, 256)
            w1t_v[pl.ds(f0, 256), :] = in_v[:, pl.ds(W1O + f0, 256)].T
            return carry

        jax.lax.fori_loop(0, F // 256, transpose_w1, 0)

        def s_tile(t, carry):
            s0 = pl.multiple_of(t * 128, 128)
            acc_v[...] = jnp.zeros((D, 128), F32)

            def f_chunk(j, c2):
                f0 = pl.multiple_of(j * 256, 256)
                h = _dot(w1t_v[pl.ds(f0, 256), :], in_v[:, pl.ds(XO + s0, 128)])
                g = (h * jax.nn.sigmoid(h)).astype(BF)
                acc_v[...] = acc_v[...] + _dot(in_v[:, pl.ds(W2O + f0, 256)], g)
                return c2

            jax.lax.fori_loop(0, F // 256, f_chunk, 0)
            o_v[:, pl.ds(s0, 128)] = acc_v[...].astype(BF)
            return carry

        jax.lax.fori_loop(0, S // 128, s_tile, 0)
        cp = pltpu.make_async_copy(o_v, o_hbm, aux_sem.at[3])
        cp.start()
        cp.wait()


@jax.jit
def pallas_standalone__dense_activation_silu__prompt_kernel(
    x: jax.Array,
    w1: jax.Array,
    w2: jax.Array,
):
    assert x.shape == (1, S, D) and w1.shape == (D, F) and w2.shape == (F, D)
    xt = x.reshape(S, D).T
    w2t = w2.T
    out_t = pl.pallas_call(
        _ffn_kernel,
        in_specs=[pl.BlockSpec(memory_space=pl.ANY)] * 3,
        out_specs=pl.BlockSpec(memory_space=pl.ANY),
        out_shape=jax.ShapeDtypeStruct((D, S), x.dtype),
        scratch_shapes=[
            pltpu.VMEM((D, WIN), BF),
            pltpu.VMEM((4, HF, HS), F32),
            pltpu.VMEM((8, HS // 128, HF, 128), BF),
            pltpu.VMEM((D, S), BF),
            pltpu.VMEM((32, WIN), F32),
            pltpu.VMEM((F, D), BF),
            pltpu.VMEM((D, 128), F32),
            pltpu.SemaphoreType.DMA((len(_PIECES),)),
            pltpu.SemaphoreType.DMA((len(_OUTS),)),
            pltpu.SemaphoreType.DMA((4,)),
        ],
        compiler_params=pltpu.CompilerParams(
            vmem_limit_bytes=110 * 1024 * 1024,
            disable_semaphore_checks=True,
            disable_bounds_checks=True,
        ),
    )(xt, w1, w2t)
    return out_t.T.reshape(1, S, D)
```
